```python
import jax
import jax.numpy as jnp

def _softmax(x, axis=-1):
    return jax.nn.softmax(x, axis=axis)
def _gelu(x):
    return jax.nn.gelu(x, approximate=True)
def _silu(x):
    return jax.nn.silu(x)
def _sigmoid(x):
    return jax.nn.sigmoid(x)
def _layernorm(x, axis=-1, eps=1e-5):
    m = jnp.mean(x, axis=axis, keepdims=True)
    v = jnp.var(x, axis=axis, keepdims=True)
    return (x - m) / jnp.sqrt(v + eps)
def _scatter_add(tgt, idx, src, axis=0):
    return tgt.at[idx].add(src)
def _segment_sum(src, seg, n):
    return jax.ops.segment_sum(src, seg, n)
class _Rng:
    def __init__(self, key):
        self._k = key
    def _next(self):
        self._k, sub = jax.random.split(self._k)
        return sub
    def normal(self, shape):
        return jax.random.normal(self._next(), shape, dtype=jnp.bfloat16)
    def randint(self, lo, hi, shape):
        return jax.random.randint(self._next(), shape, lo, hi, dtype=jnp.int32)
    def uniform(self, shape, lo=0.0, hi=1.0):
        return jax.random.uniform(self._next(), shape, jnp.bfloat16, lo, hi)
    def permutation(self, n):
        return jax.random.permutation(self._next(), n)


kernel_name = 'standalone__layernorm_linear__prompt'

def setup_inputs():
    _rng = _Rng(jax.random.key(int.from_bytes(__import__("os").urandom(4), "little")))
    _w = (lambda a: (lambda t: t.astype(jnp.bfloat16) if jnp.issubdtype(t.dtype, jnp.floating) else t)(jnp.asarray(a)))
    B, S, D = 2, 2048, 1024
    return {
        "x": _w((lambda *s: _rng.normal(s) * 0.05)(B, S, D)),
        "g": _w((lambda *s: _rng.normal(s) * 0.05)(D) + 1.0),
        "b": _w((lambda *s: _rng.normal(s) * 0.05)(D)),
        "w": _w((lambda *s: _rng.normal(s) * 0.05)(D, D)),
    }

def reference(x, g, b, w):
    return (_layernorm(x, axis=-1) * g + b) @ w
```

```python
import jax
import jax.numpy as jnp
import jax.experimental.pallas as pl
import jax.experimental.pallas.tpu as pltpu

_EPS = 1e-5
_M, _D, _N = 4096, 1024, 1024

_REGIONS = (256,) * 16
_XSIZES = (256, 256, 256, 1024, 2304)
_WSIZES = (256, 256, 256, 256)
_NT = 256
_LNSUB = 32


def _ln_rows(x_bf16, g32, b32):
    x = x_bf16.astype(jnp.float32)
    m = jnp.mean(x, axis=-1, keepdims=True)
    xc = x - m
    v = jnp.mean(xc * xc, axis=-1, keepdims=True)
    y = xc * jax.lax.rsqrt(v + _EPS) * g32 + b32
    return y.astype(jnp.bfloat16)


def _schedule():
    regions, nt, lnsub = _REGIONS, _NT, _LNSUB
    n = len(regions)
    rs = [0]
    for r in regions:
        rs.append(rs[-1] + r)
    xch, r = [], 0
    for s in _XSIZES:
        xch.append((r, s))
        r += s
    wch, c = [], 0
    for s in _WSIZES:
        wch.append((c, s))
        c += s
    och = [(rs[j], regions[j], 0, _N) for j in range(n - 1)]
    och += [(rs[n - 1], regions[n - 1], s * nt, nt) for s in range(_N // nt)]

    ops = [("gstart",), ("fence",), ("xstart", 0)]
    ops += [("wstart", p) for p in range(len(wch))]
    ops += [("xstart", i) for i in range(1, len(xch))]
    ops += [("xwait", 0), ("gwait",)]
    xw, ww = {0}, set()

    def need_x(r0, nr):
        for i, (a, _) in enumerate(xch):
            if i not in xw and a < r0 + nr:
                ops.append(("xwait", i))
                xw.add(i)

    def need_w(n0, nn):
        for i, (a, _) in enumerate(wch):
            if i not in ww and a < n0 + nn:
                ops.append(("wwait", i))
                ww.add(i)

    ops += [("ln", s * lnsub, lnsub) for s in range(regions[0] // lnsub)]
    nmm = _N // nt
    for j in range(n):
        lq = []
        if j + 1 < n:
            lq = [rs[j + 1] + s * lnsub for s in range(regions[j + 1] // lnsub)]
        per = -(-len(lq) // nmm)
        if j >= 1 and j + 1 < n:
            need_x(rs[j + 1], regions[j + 1])
        for s in range(nmm):
            need_w(s * nt, nt)
            if j > 0:
                for _ in range(per):
                    if lq:
                        ops.append(("ln", lq.pop(0), lnsub))
            ops.append(("mm", rs[j], regions[j], s * nt, nt))
            if j == n - 1:
                ops.append(("ostart", n - 1 + s))
            if s == 0 and j >= 1:
                ops.append(("ostart", j - 1))
        if j == 0 and lq:
            need_x(rs[1], regions[1])
            while lq:
                ops.append(("ln", lq.pop(0), lnsub))
    ops += [("owait", i) for i in range(len(och))]
    return ops, xch, wch, och


def _make_kernel(ops, xch, wch, och):
    xo = _D

    def kernel(x_hbm, g_hbm, b_hbm, w_hbm, o_hbm,
               xw_vmem, y_vmem, o_vmem, g_vmem, b_vmem, xs, ws, os_, gs, fsem):
        def xcp(i):
            r0, nr = xch[i]
            return pltpu.make_async_copy(
                x_hbm.at[pl.ds(r0, nr)], xw_vmem.at[pl.ds(xo + r0, nr)], xs.at[i])

        def wcp(i):
            n0, nn = wch[i]
            return pltpu.make_async_copy(
                w_hbm.at[:, pl.ds(n0, nn)], xw_vmem.at[pl.ds(0, _D), pl.ds(n0, nn)], ws.at[i])

        def ocp(i):
            r0, nr, n0, nn = och[i]
            return pltpu.make_async_copy(
                o_vmem.at[pl.ds(r0, nr), pl.ds(n0, nn)],
                o_hbm.at[pl.ds(r0, nr), pl.ds(n0, nn)], os_.at[i])

        gcp = pltpu.make_async_copy(g_hbm, g_vmem, gs.at[0])
        bcp = pltpu.make_async_copy(b_hbm, b_vmem, gs.at[1])
        g32 = b32 = None
        for op in ops:
            k = op[0]
            if k == "xstart":
                xcp(op[1]).start()
            elif k == "xwait":
                xcp(op[1]).wait()
            elif k == "wstart":
                wcp(op[1]).start()
            elif k == "wwait":
                wcp(op[1]).wait()
            elif k == "ostart":
                ocp(op[1]).start()
            elif k == "owait":
                ocp(op[1]).wait()
            elif k == "gstart":
                gcp.start()
                bcp.start()
            elif k == "fence":
                pl.semaphore_signal(fsem, 1)
                pl.semaphore_wait(fsem, 1)
            elif k == "gwait":
                gcp.wait()
                bcp.wait()
                g32 = g_vmem[...].astype(jnp.float32).reshape(1, _D)
                b32 = b_vmem[...].astype(jnp.float32).reshape(1, _D)
            elif k == "ln":
                _, r0, nr = op
                y = _ln_rows(xw_vmem[pl.ds(xo + r0, nr), :], g32, b32)
                y_vmem[pl.ds(r0 // 2, nr // 2), :] = pltpu.bitcast(y, jnp.uint32)
            elif k == "mm":
                _, r0, nr, n0, nn = op
                a = pltpu.bitcast(y_vmem[pl.ds(r0 // 2, nr // 2), :], jnp.bfloat16)
                o_vmem[pl.ds(r0, nr), pl.ds(n0, nn)] = jnp.dot(
                    a, xw_vmem[pl.ds(0, _D), pl.ds(n0, nn)],
                    preferred_element_type=jnp.float32).astype(jnp.bfloat16)
            else:
                raise ValueError(op)

    return kernel


@jax.jit
def pallas_standalone__layernorm_linear__prompt_kernel(x, g, b, w):
    bsz, seq, d = x.shape
    assert (bsz * seq, d, w.shape[1]) == (_M, _D, _N)
    ops, xch, wch, och = _schedule()
    anyspec = pl.BlockSpec(memory_space=pl.ANY)
    out = pl.pallas_call(
        _make_kernel(ops, xch, wch, och),
        grid=(),
        in_specs=[anyspec] * 4,
        out_specs=anyspec,
        out_shape=jax.ShapeDtypeStruct((_M, _N), x.dtype),
        scratch_shapes=[
            pltpu.VMEM((_D + _M, _D), jnp.bfloat16),
            pltpu.VMEM((_M // 2, _D), jnp.uint32),
            pltpu.VMEM((_M, _N), jnp.bfloat16),
            pltpu.VMEM((_D,), jnp.bfloat16),
            pltpu.VMEM((_D,), jnp.bfloat16),
            pltpu.SemaphoreType.DMA((len(xch),)),
            pltpu.SemaphoreType.DMA((len(wch),)),
            pltpu.SemaphoreType.DMA((len(och),)),
            pltpu.SemaphoreType.DMA((2,)),
            pltpu.SemaphoreType.REGULAR,
        ],
        compiler_params=pltpu.CompilerParams(
            vmem_limit_bytes=64 * 1024 * 1024,
            flags={"XLA_TPU_EVENLY_DISTRIBUTE_CRITICAL_NODES": True},
        ),
        name="layernorm_linear",
    )(x.reshape(_M, _D), g, b, w)
    return out.reshape(bsz, seq, _N)
```

```python
import jax
import jax.numpy as jnp
import jax.experimental.pallas as pl
import jax.experimental.pallas.tpu as pltpu

_EPS = 1e-5
_M, _D, _N = 4096, 1024, 1024
_H = 512
_G = 16

_REGIONS = (256,) * 7 + (128, 128)
_XSIZES = (128, 128, 128, 128, 512, 512, 512, 2048)
_NT, _TAIL_NT = 256, 128
_LNROWS = 32
_PREPSUB = 128
_ORDER = (2, 5, 1, 3, 6, 4, 7)

_QUAD = {0: (0, 0), 1: (0, _H), 2: (_H, 0), 3: (_H, _H)}
_SBSLOT = {1: 0, 3: 1, 4: 2, 6: 3, 7: 4}
_PREP = {1: (0, 3, 1), 3: (1, 3, -1), 4: (2, 0, -1), 6: (0, 1, 1), 7: (2, 3, 1)}

_f32, _bf16, _u32 = jnp.float32, jnp.bfloat16, jnp.uint32


def _ln_f32(x_bf16, g32, b32):
    x = x_bf16.astype(_f32)
    m = jnp.mean(x, axis=-1, keepdims=True)
    xc = x - m
    v = jnp.mean(xc * xc, axis=-1, keepdims=True)
    return xc * jax.lax.rsqrt(v + _EPS) * g32 + b32


def _pack(v):
    return pltpu.bitcast(v.astype(_bf16), _u32)


def _schedule():
    regions, n = _REGIONS, len(_REGIONS)
    ps = [0]
    for r in regions:
        ps.append(ps[-1] + 2 * r)
    xch, r = [], 0
    for s in _XSIZES:
        xch.append((r, s))
        r += s
    och = [(ps[j], 2 * regions[j], 0, _N) for j in range(n - 1)]
    tail_idx = {}
    for c in range(_H // _TAIL_NT):
        tail_idx[(6, c)] = len(och)
        och.append((ps[n - 1], 2 * regions[-1], _H + c * _TAIL_NT, _TAIL_NT))
        tail_idx[(7, c)] = len(och)
        och.append((ps[n - 1], 2 * regions[-1], c * _TAIL_NT, _TAIL_NT))

    first_x = [i for i, (a, _) in enumerate(xch) if a < ps[1]]
    ops = [("gstart",), ("fence",)] + [("xstart", i) for i in first_x]
    ops += [("wstart", q) for q in (0, 3, 1, 2)]
    ops += [("xstart", i) for i in range(len(xch)) if i not in first_x]
    xw = set()

    def need_x(r0, nr):
        for i, (a, _) in enumerate(xch):
            if i not in xw and a < r0 + nr:
                ops.append(("xwait", i))
                xw.add(i)

    def ln_list(j):
        return [("ln", ps[j] + s0, _LNROWS // 2) for s0 in range(0, 2 * regions[j], _LNROWS)]

    def preps(i):
        return [("prep", i, k0, _PREPSUB) for k0 in range(0, _H, _PREPSUB)]

    for t, o in enumerate(ln_list(0)):
        need_x(o[1], 2 * o[2])
        if t == 0:
            ops.append(("gwait",))
        ops.append(o)

    for j in range(n):
        rj = regions[j]
        ntj = _TAIL_NT if j == n - 1 else _NT
        cn = _H // ntj
        lq = ln_list(j + 1) if j + 1 < n else []
        if j == 0:
            waits = {2: [0], 5: [3], 3: [1], 4: [2]}
            seq = [(i, c) for i in _ORDER for c in range(cn)]
            start = [t for t, (i, c) in enumerate(seq) if i == 4][0]
            per, done = len(lq) / (len(seq) - start), 0
            for t, (i, c) in enumerate(seq):
                if c == 0:
                    ops.extend(("wwait", q) for q in waits.get(i, []))
                    if t == start:
                        need_x(ps[1], 2 * regions[1])
                    if i in _PREP:
                        ops.extend(preps(i))
                if t >= start:
                    while lq and done < (t - start + 1) * per:
                        ops.append(lq.pop(0))
                        done += 1
                ops.append(("mm", i, ps[j], rj, c, ntj, j % 2))
            continue
        if lq:
            need_x(ps[j + 1], 2 * regions[j + 1])
        seq = [(i, c) for c in range(cn) for i in _ORDER]
        per, done = len(lq) / len(seq), 0
        for t, (i, c) in enumerate(seq):
            while lq and done < (t + 1) * per:
                ops.append(lq.pop(0))
                done += 1
            ops.append(("mm", i, ps[j], rj, c, ntj, j % 2))
            if t == 0:
                ops.append(("ostart", j - 1))
            if j == n - 1 and (i, c) in tail_idx:
                ops.append(("ostart", tail_idx[(i, c)]))
    ops += [("owait", i) for i in range(len(och))]
    return ops, xch, och


def _make_kernel(ops, xch, och):
    xo = _D

    def kernel(x_hbm, g_hbm, b_hbm, w_hbm, o_hbm,
               xw_vmem, sa_vmem, sb_vmem, t_vmem, o_vmem, g_vmem, b_vmem,
               xs, ws, os_, gs, fsem):
        def xcp(i):
            r0, nr = xch[i]
            return pltpu.make_async_copy(
                x_hbm.at[pl.ds(r0, nr)], xw_vmem.at[pl.ds(xo + r0, nr)], xs.at[i])

        def wcp(q):
            r0, c0 = _QUAD[q]
            return pltpu.make_async_copy(
                w_hbm.at[pl.ds(r0, _H), pl.ds(c0, _H)],
                xw_vmem.at[pl.ds(r0, _H), pl.ds(c0, _H)], ws.at[q])

        def ocp(i):
            r0, nr, n0, nn = och[i]
            return pltpu.make_async_copy(
                o_vmem.at[pl.ds(r0, nr), pl.ds(n0, nn)],
                o_hbm.at[pl.ds(r0, nr), pl.ds(n0, nn)], os_.at[i])

        def wq(q, k0, nk):
            r0, c0 = _QUAD[q]
            return xw_vmem[pl.ds(r0 + k0, nk), pl.ds(c0, _H)].astype(_f32)

        def prod(i, p0, r, c, nt):
            a = pltpu.bitcast(sa_vmem[i - 1, pl.ds(p0 // 4, r // 2), :], _bf16)
            if i == 2:
                bb = xw_vmem[pl.ds(0, _H), pl.ds(c * nt, nt)]
            elif i == 5:
                bb = xw_vmem[pl.ds(_H, _H), pl.ds(_H + c * nt, nt)]
            else:
                bb = pltpu.bitcast(sb_vmem[_SBSLOT[i], :, pl.ds(c * nt, nt)], _bf16)
            return jnp.dot(a, bb, preferred_element_type=_f32)

        def put(val, p0, r, isq, cols):
            v = val.astype(_bf16)
            for i in range(r // _G):
                o_vmem[pl.ds(p0 + (2 * i + isq) * _G, _G), cols] = v[i * _G:(i + 1) * _G]

        gcp = pltpu.make_async_copy(g_hbm, g_vmem, gs.at[0])
        bcp = pltpu.make_async_copy(b_hbm, b_vmem, gs.at[1])
        g32 = b32 = None
        for op in ops:
            k = op[0]
            if k == "xstart":
                xcp(op[1]).start()
            elif k == "xwait":
                xcp(op[1]).wait()
            elif k == "wstart":
                wcp(op[1]).start()
            elif k == "wwait":
                wcp(op[1]).wait()
            elif k == "ostart":
                ocp(op[1]).start()
            elif k == "owait":
                ocp(op[1]).wait()
            elif k == "gstart":
                gcp.start()
                bcp.start()
            elif k == "fence":
                pl.semaphore_signal(fsem, 1)
                pl.semaphore_wait(fsem, 1)
            elif k == "gwait":
                gcp.wait()
                bcp.wait()
                g32 = g_vmem[...].astype(_f32).reshape(1, _D)
                b32 = b_vmem[...].astype(_f32).reshape(1, _D)
            elif k == "prep":
                _, i, k0, nk = op
                qa, qb, sign = _PREP[i]
                wa, wb = wq(qa, k0, nk), wq(qb, k0, nk)
                sb_vmem[_SBSLOT[i], pl.ds(k0 // 2, nk // 2), :] = _pack(
                    wa + wb if sign > 0 else wa - wb)
            elif k == "ln":
                _, r0, nr = op
                for gi in range(nr // _G):
                    rr = r0 + 2 * gi * _G
                    yp = _ln_f32(xw_vmem[pl.ds(xo + rr, _G), :], g32, b32)
                    yq = _ln_f32(xw_vmem[pl.ds(xo + rr + _G, _G), :], g32, b32)
                    a11, a12, a21, a22 = yp[:, :_H], yp[:, _H:], yq[:, :_H], yq[:, _H:]
                    lhs = (a11 + a22, a21 + a22, a11, a22, a11 + a12, a21 - a11, a12 - a22)
                    for i in range(7):
                        sa_vmem[i, pl.ds(rr // 4, _G // 2), :] = _pack(lhs[i])
            elif k == "mm":
                _, i, p0, r, c, nt, tb = op
                m = prod(i, p0, r, c, nt)
                left, right = pl.ds(c * nt, nt), pl.ds(_H + c * nt, nt)
                t11, t12, t21, t22 = (
                    t_vmem.at[tb * 4 + t, pl.ds(0, r), left] for t in range(4))
                if i == 2:
                    t21[...] = m
                    t22[...] = -m
                elif i == 5:
                    t12[...] = m
                    t11[...] = -m
                elif i == 1:
                    t11[...] = t11[...] + m
                    t22[...] = t22[...] + m
                elif i == 3:
                    put(t12[...] + m, p0, r, 0, right)
                    t22[...] = t22[...] + m
                elif i == 6:
                    put(t22[...] + m, p0, r, 1, right)
                elif i == 4:
                    put(t21[...] + m, p0, r, 1, left)
                    t11[...] = t11[...] + m
                elif i == 7:
                    put(t11[...] + m, p0, r, 0, left)
            else:
                raise ValueError(op)

    return kernel


@jax.jit
def pallas_standalone__layernorm_linear__prompt_kernel(x, g, b, w):
    bsz, seq, d = x.shape
    assert (bsz * seq, d, w.shape[1]) == (_M, _D, _N)
    ops, xch, och = _schedule()
    anyspec = pl.BlockSpec(memory_space=pl.ANY)
    out = pl.pallas_call(
        _make_kernel(ops, xch, och),
        grid=(),
        in_specs=[anyspec] * 4,
        out_specs=anyspec,
        out_shape=jax.ShapeDtypeStruct((_M, _N), x.dtype),
        scratch_shapes=[
            pltpu.VMEM((_D + _M, _D), _bf16),
            pltpu.VMEM((7, _M // 4, _H), _u32),
            pltpu.VMEM((5, _H // 2, _H), _u32),
            pltpu.VMEM((8, max(_REGIONS), _H), _f32),
            pltpu.VMEM((_M, _N), _bf16),
            pltpu.VMEM((_D,), _bf16),
            pltpu.VMEM((_D,), _bf16),
            pltpu.SemaphoreType.DMA((len(xch),)),
            pltpu.SemaphoreType.DMA((4,)),
            pltpu.SemaphoreType.DMA((len(och),)),
            pltpu.SemaphoreType.DMA((2,)),
            pltpu.SemaphoreType.REGULAR,
        ],
        compiler_params=pltpu.CompilerParams(
            vmem_limit_bytes=64 * 1024 * 1024,
            flags={"XLA_TPU_EVENLY_DISTRIBUTE_CRITICAL_NODES": True},
        ),
        name="layernorm_linear",
    )(x.reshape(_M, _D), g, b, w)
    return out.reshape(bsz, seq, _N)
```

```python
import jax
import jax.numpy as jnp
import jax.experimental.pallas as pl
import jax.experimental.pallas.tpu as pltpu

_EPS = 1e-5
_M, _D, _N = 4096, 1024, 1024
_H = 512
_G = 16

_REGIONS = (256, 128) + (256,) * 6 + (128,)
_XSIZES = (128, 128, 128, 128, 256, 512, 512, 512, 1792)
_NT, _TAIL_NT = 256, 128
_LNROWS = 32
_ORDER = (2, 5, 1, 3, 6, 4, 7)

_QUAD = {0: (0, 0), 1: (0, _H), 2: (_H, 0), 3: (_H, _H)}
_SBSLOT = {1: 0, 3: 1, 4: 2, 6: 3, 7: 4}
_PREP = {1: (0, 3, 1), 3: (1, 3, -1), 4: (2, 0, -1), 6: (0, 1, 1), 7: (2, 3, 1)}

_f32, _bf16, _u32 = jnp.float32, jnp.bfloat16, jnp.uint32


def _ln_f32(x, g32, b32):
    m = jnp.mean(x, axis=-1, keepdims=True)
    xc = x - m
    v = jnp.mean(xc * xc, axis=-1, keepdims=True)
    return xc * jax.lax.rsqrt(v + _EPS) * g32 + b32


def _unpack(words):
    return [pltpu.unpack_elementwise(words, index=h, packed_dtype=_bf16, unpacked_dtype=_f32)
            for h in range(2)]


def _pack(even, odd):
    return pltpu.pack_elementwise([even, odd], packed_dtype=_bf16)


def _schedule():
    regions, n = _REGIONS, len(_REGIONS)
    ps = [0]
    for r in regions:
        ps.append(ps[-1] + 2 * r)
    xch, r = [], 0
    for s in _XSIZES:
        xch.append((r, s))
        r += s
    och = [(ps[j], 2 * regions[j], 0, _N) for j in range(n - 1)]
    tail_idx = {}
    for c in range(_H // _TAIL_NT):
        tail_idx[(6, c)] = len(och)
        och.append((ps[n - 1], 2 * regions[-1], _H + c * _TAIL_NT, _TAIL_NT))
        tail_idx[(7, c)] = len(och)
        och.append((ps[n - 1], 2 * regions[-1], c * _TAIL_NT, _TAIL_NT))

    wch, wid = [], {}
    for c in range(_H // _NT):
        for q in (0, 3, 1, 2):
            wid[(q, c)] = len(wch)
            wch.append((_QUAD[q][0], _QUAD[q][1] + c * _NT, _H, _NT))
    first_x = [i for i, (a, _) in enumerate(xch) if a < ps[1]]
    second_x = [i for i, (a, _) in enumerate(xch) if ps[1] <= a < ps[2]]
    ops = [("gstart",), ("fence",)] + [("xstart", i) for i in first_x]
    ops += [("wstart", wid[(q, 0)]) for q in (0, 3, 1, 2)]
    ops += [("xstart", i) for i in second_x]
    for c in range(1, _H // _NT):
        ops += [("wstart", wid[(q, c)]) for q in (0, 3, 1, 2)]
    ops += [("xstart", i) for i in range(len(xch)) if i not in first_x + second_x]
    xw = set()

    def need_x(r0, nr):
        for i, (a, _) in enumerate(xch):
            if i not in xw and a < r0 + nr:
                ops.append(("xwait", i))
                xw.add(i)

    def ln_list(j):
        return [("ln", ps[j] + s0, _LNROWS // 2) for s0 in range(0, 2 * regions[j], _LNROWS)]

    for t, o in enumerate(ln_list(0)):
        need_x(o[1], 2 * o[2])
        if t == 0:
            ops.append(("gwait",))
        ops.append(o)

    for j in range(n):
        rj = regions[j]
        ntj = _TAIL_NT if j == n - 1 else _NT
        lq = ln_list(j + 1) if j + 1 < n else []
        seq = [(i, c) for c in range(_H // ntj) for i in _ORDER]
        if j == 0:
            start = len(_ORDER)
            per, done = len(lq) / (len(seq) - start), 0
            for t, (i, c) in enumerate(seq):
                if c == 0:
                    quads = {2: (0,), 5: (3,), 3: (1,), 4: (2,)}.get(i, ())
                else:
                    quads = {2: (0, 3), 3: (1, 2)}.get(i, ())
                ops.extend(("wwait", wid[(q, c)]) for q in quads)
                if t == start:
                    need_x(ps[1], 2 * regions[1])
                if i in _PREP:
                    ops.append(("prep", i, c * ntj, ntj))
                if t >= start:
                    while lq and done < (t - start + 1) * per:
                        ops.append(lq.pop(0))
                        done += 1
                ops.append(("mm", i, ps[j], rj, c, ntj, j % 2))
            continue
        if lq:
            need_x(ps[j + 1], 2 * regions[j + 1])
        per, done = len(lq) / len(seq), 0
        for t, (i, c) in enumerate(seq):
            while lq and done < (t + 1) * per:
                ops.append(lq.pop(0))
                done += 1
            ops.append(("mm", i, ps[j], rj, c, ntj, j % 2))
            if t == 0:
                ops.append(("ostart", j - 1))
            if j == n - 1 and (i, c) in tail_idx:
                ops.append(("ostart", tail_idx[(i, c)]))
    ops += [("owait", i) for i in range(len(och))]
    return ops, xch, wch, och


def _make_kernel(ops, xch, wch, och):
    xo = _D

    def kernel(x_hbm, g_hbm, b_hbm, w_hbm, o_hbm,
               xw_vmem, sa_vmem, sb_vmem, t_vmem, o_vmem, g_vmem, b_vmem,
               xs, ws, os_, gs, fsem):
        x32_hbm, w32_hbm = x_hbm.bitcast(_u32), w_hbm.bitcast(_u32)

        def xcp(i):
            r0, nr = xch[i]
            return pltpu.make_async_copy(
                x32_hbm.at[pl.ds(r0 // 2, nr // 2)],
                xw_vmem.at[pl.ds((xo + r0) // 2, nr // 2)], xs.at[i])

        def wcp(i):
            r0, c0, nr, nc = wch[i]
            return pltpu.make_async_copy(
                w32_hbm.at[pl.ds(r0 // 2, nr // 2), pl.ds(c0, nc)],
                xw_vmem.at[pl.ds(r0 // 2, nr // 2), pl.ds(c0, nc)], ws.at[i])

        def ocp(i):
            r0, nr, n0, nn = och[i]
            return pltpu.make_async_copy(
                o_vmem.at[pl.ds(r0, nr), pl.ds(n0, nn)],
                o_hbm.at[pl.ds(r0, nr), pl.ds(n0, nn)], os_.at[i])

        def wq(q, n0, nn):
            r0, c0 = _QUAD[q]
            return xw_vmem[pl.ds(r0 // 2, _H // 2), pl.ds(c0 + n0, nn)]

        def prod(i, p0, r, c, nt):
            a = pltpu.bitcast(sa_vmem[i - 1, pl.ds(p0 // 4, r // 2), :], _bf16)
            if i == 2:
                bb = wq(0, c * nt, nt)
            elif i == 5:
                bb = wq(3, c * nt, nt)
            else:
                bb = sb_vmem[_SBSLOT[i], :, pl.ds(c * nt, nt)]
            return jnp.dot(a, pltpu.bitcast(bb, _bf16), preferred_element_type=_f32)

        def put(val, p0, r, isq, cols):
            for i in range(r // _G):
                o_vmem[pl.ds(p0 + (2 * i + isq) * _G, _G), cols] = (
                    val[i * _G:(i + 1) * _G].astype(_bf16))

        gcp = pltpu.make_async_copy(g_hbm, g_vmem, gs.at[0])
        bcp = pltpu.make_async_copy(b_hbm, b_vmem, gs.at[1])
        g32 = b32 = None
        for op in ops:
            k = op[0]
            if k == "xstart":
                xcp(op[1]).start()
            elif k == "xwait":
                xcp(op[1]).wait()
            elif k == "wstart":
                wcp(op[1]).start()
            elif k == "wwait":
                wcp(op[1]).wait()
            elif k == "ostart":
                ocp(op[1]).start()
            elif k == "owait":
                ocp(op[1]).wait()
            elif k == "gstart":
                gcp.start()
                bcp.start()
            elif k == "fence":
                pl.semaphore_signal(fsem, 1)
                pl.semaphore_wait(fsem, 1)
            elif k == "gwait":
                gcp.wait()
                bcp.wait()
                g32 = g_vmem[...].astype(_f32).reshape(1, _D)
                b32 = b_vmem[...].astype(_f32).reshape(1, _D)
            elif k == "prep":
                _, i, n0, nn = op
                qa, qb, sign = _PREP[i]
                wa, wb = _unpack(wq(qa, n0, nn)), _unpack(wq(qb, n0, nn))
                sb_vmem[_SBSLOT[i], :, pl.ds(n0, nn)] = _pack(
                    *[wa[h] + wb[h] if sign > 0 else wa[h] - wb[h] for h in range(2)])
            elif k == "ln":
                _, r0, nr = op
                for gi in range(nr // _G):
                    rr = r0 + 2 * gi * _G
                    xp = _unpack(xw_vmem[pl.ds((xo + rr) // 2, _G // 2), :])
                    xq = _unpack(xw_vmem[pl.ds((xo + rr + _G) // 2, _G // 2), :])
                    lhs = []
                    for h in range(2):
                        yp, yq = _ln_f32(xp[h], g32, b32), _ln_f32(xq[h], g32, b32)
                        a11, a12, a21, a22 = yp[:, :_H], yp[:, _H:], yq[:, :_H], yq[:, _H:]
                        lhs.append((a11 + a22, a21 + a22, a11, a22,
                                    a11 + a12, a21 - a11, a12 - a22))
                    for i in range(7):
                        sa_vmem[i, pl.ds(rr // 4, _G // 2), :] = _pack(lhs[0][i], lhs[1][i])
            elif k == "mm":
                _, i, p0, r, c, nt, tb = op
                m = prod(i, p0, r, c, nt)
                left, right = pl.ds(c * nt, nt), pl.ds(_H + c * nt, nt)
                t11, t12, t21, t22 = (
                    t_vmem.at[tb * 4 + t, pl.ds(0, r), left] for t in range(4))
                if i == 2:
                    t21[...] = m
                    t22[...] = -m
                elif i == 5:
                    t12[...] = m
                    t11[...] = -m
                elif i == 1:
                    t11[...] = t11[...] + m
                    t22[...] = t22[...] + m
                elif i == 3:
                    put(t12[...] + m, p0, r, 0, right)
                    t22[...] = t22[...] + m
                elif i == 6:
                    put(t22[...] + m, p0, r, 1, right)
                elif i == 4:
                    put(t21[...] + m, p0, r, 1, left)
                    t11[...] = t11[...] + m
                elif i == 7:
                    put(t11[...] + m, p0, r, 0, left)
            else:
                raise ValueError(op)

    return kernel


@jax.jit
def pallas_standalone__layernorm_linear__prompt_kernel(x, g, b, w):
    bsz, seq, d = x.shape
    assert (bsz * seq, d, w.shape[1]) == (_M, _D, _N)
    ops, xch, wch, och = _schedule()
    anyspec = pl.BlockSpec(memory_space=pl.ANY)
    out = pl.pallas_call(
        _make_kernel(ops, xch, wch, och),
        grid=(),
        in_specs=[anyspec] * 4,
        out_specs=anyspec,
        out_shape=jax.ShapeDtypeStruct((_M, _N), x.dtype),
        scratch_shapes=[
            pltpu.VMEM(((_D + _M) // 2, _D), _u32),
            pltpu.VMEM((7, _M // 4, _H), _u32),
            pltpu.VMEM((5, _H // 2, _H), _u32),
            pltpu.VMEM((8, max(_REGIONS), _H), _f32),
            pltpu.VMEM((_M, _N), _bf16),
            pltpu.VMEM((_D,), _bf16),
            pltpu.VMEM((_D,), _bf16),
            pltpu.SemaphoreType.DMA((len(xch),)),
            pltpu.SemaphoreType.DMA((len(wch),)),
            pltpu.SemaphoreType.DMA((len(och),)),
            pltpu.SemaphoreType.DMA((2,)),
            pltpu.SemaphoreType.REGULAR,
        ],
        compiler_params=pltpu.CompilerParams(
            vmem_limit_bytes=64 * 1024 * 1024,
            flags={"XLA_TPU_EVENLY_DISTRIBUTE_CRITICAL_NODES": True},
        ),
        name="layernorm_linear",
    )(x.reshape(_M, _D), g, b, w)
    return out.reshape(bsz, seq, _N)
```

```python
import jax
import jax.numpy as jnp
import jax.experimental.pallas as pl
import jax.experimental.pallas.tpu as pltpu

_EPS = 1e-5
_M, _D, _N = 4096, 1024, 1024
_H = 512
_G = 16

_REGIONS = (256, 128) + (256,) * 6 + (64, 64)
_XSIZES = (128, 128, 128, 128, 256, 512, 512, 512, 1792)
_NT0, _NT, _TAIL_NT = 256, 512, 128
_LNROWS = 32
_ORDER = (2, 5, 1, 3, 6, 4, 7)

_QUAD = {0: (0, 0), 1: (0, _H), 2: (_H, 0), 3: (_H, _H)}
_SBSLOT = {1: 0, 3: 1, 4: 2, 6: 3, 7: 4}
_PREP = {1: (0, 3, 1), 3: (1, 3, -1), 4: (2, 0, -1), 6: (0, 1, 1), 7: (2, 3, 1)}

_f32, _bf16, _u32 = jnp.float32, jnp.bfloat16, jnp.uint32


def _ln_f32(x, g32, b32):
    m = jnp.mean(x, axis=-1, keepdims=True)
    xc = x - m
    v = jnp.mean(xc * xc, axis=-1, keepdims=True)
    return xc * jax.lax.rsqrt(v + _EPS) * g32 + b32


def _unpack(words):
    return [pltpu.unpack_elementwise(words, index=h, packed_dtype=_bf16, unpacked_dtype=_f32)
            for h in range(2)]


def _pack(even, odd):
    return pltpu.pack_elementwise([even, odd], packed_dtype=_bf16)


def _schedule():
    regions, n = _REGIONS, len(_REGIONS)
    ps = [0]
    for r in regions:
        ps.append(ps[-1] + 2 * r)
    xch, r = [], 0
    for s in _XSIZES:
        xch.append((r, s))
        r += s
    och = [(ps[j], 2 * regions[j], 0, _N) for j in range(n - 1)]
    tail_idx = {}
    for c in range(_H // _TAIL_NT):
        tail_idx[(6, c)] = len(och)
        och.append((ps[n - 1], 2 * regions[-1], _H + c * _TAIL_NT, _TAIL_NT))
        tail_idx[(7, c)] = len(och)
        och.append((ps[n - 1], 2 * regions[-1], c * _TAIL_NT, _TAIL_NT))

    wch, wid = [], {}
    for c in range(_H // _NT0):
        for q in (0, 3, 1, 2):
            wid[(q, c)] = len(wch)
            wch.append((_QUAD[q][0], _QUAD[q][1] + c * _NT0, _H, _NT0))
    first_x = [i for i, (a, _) in enumerate(xch) if a < ps[1]]
    second_x = [i for i, (a, _) in enumerate(xch) if ps[1] <= a < ps[2]]
    ops = [("gstart",), ("fence",)] + [("xstart", i) for i in first_x]
    ops += [("wstart", wid[(q, 0)]) for q in (0, 3, 1, 2)]
    ops += [("xstart", i) for i in second_x]
    for c in range(1, _H // _NT0):
        ops += [("wstart", wid[(q, c)]) for q in (0, 3, 1, 2)]
    ops += [("xstart", i) for i in range(len(xch)) if i not in first_x + second_x]
    xw = set()

    def need_x(r0, nr):
        for i, (a, _) in enumerate(xch):
            if i not in xw and a < r0 + nr:
                ops.append(("xwait", i))
                xw.add(i)

    def ln_list(j):
        return [("ln", ps[j] + s0, _LNROWS // 2) for s0 in range(0, 2 * regions[j], _LNROWS)]

    for t, o in enumerate(ln_list(0)):
        need_x(o[1], 2 * o[2])
        if t == 0:
            ops.append(("gwait",))
        ops.append(o)

    for j in range(n):
        rj = regions[j]
        ntj = _NT0 if j == 0 else _TAIL_NT if j == n - 1 else _NT
        lq = ln_list(j + 1) if j + 1 < n else []
        seq = [(i, c) for c in range(_H // ntj) for i in _ORDER]
        if j == 0:
            start = len(_ORDER)
            per, done = len(lq) / (len(seq) - start), 0
            for t, (i, c) in enumerate(seq):
                if c == 0:
                    quads = {2: (0,), 5: (3,), 3: (1, 2)}.get(i, ())
                else:
                    quads = {2: (0, 3), 3: (1, 2)}.get(i, ())
                ops.extend(("wwait", wid[(q, c)]) for q in quads)
                if t == start:
                    need_x(ps[1], 2 * regions[1])
                if i in _PREP:
                    ops.append(("prep", i, c * ntj, ntj))
                if t >= start:
                    while lq and done < (t - start + 1) * per:
                        ops.append(lq.pop(0))
                        done += 1
                ops.append(("mm", i, ps[j], rj, c, ntj, j % 2))
            continue
        if lq:
            need_x(ps[j + 1], 2 * regions[j + 1])
        per, done = len(lq) / len(seq), 0
        for t, (i, c) in enumerate(seq):
            while lq and done < (t + 1) * per:
                ops.append(lq.pop(0))
                done += 1
            ops.append(("mm", i, ps[j], rj, c, ntj, j % 2))
            if t == 0:
                ops.append(("ostart", j - 1))
            if j == n - 1 and (i, c) in tail_idx:
                ops.append(("ostart", tail_idx[(i, c)]))
    ops += [("owait", i) for i in range(len(och))]
    return ops, xch, wch, och


def _make_kernel(ops, xch, wch, och):
    xo = _D

    def kernel(x_hbm, g_hbm, b_hbm, w_hbm, o_hbm,
               xw_vmem, sa_vmem, sb_vmem, t_vmem, o_vmem, g_vmem, b_vmem,
               xs, ws, os_, gs, fsem):
        x32_hbm, w32_hbm = x_hbm.bitcast(_u32), w_hbm.bitcast(_u32)

        def xcp(i):
            r0, nr = xch[i]
            return pltpu.make_async_copy(
                x32_hbm.at[pl.ds(r0 // 2, nr // 2)],
                xw_vmem.at[pl.ds((xo + r0) // 2, nr // 2)], xs.at[i])

        def wcp(i):
            r0, c0, nr, nc = wch[i]
            return pltpu.make_async_copy(
                w32_hbm.at[pl.ds(r0 // 2, nr // 2), pl.ds(c0, nc)],
                xw_vmem.at[pl.ds(r0 // 2, nr // 2), pl.ds(c0, nc)], ws.at[i])

        def ocp(i):
            r0, nr, n0, nn = och[i]
            return pltpu.make_async_copy(
                o_vmem.at[pl.ds(r0, nr), pl.ds(n0, nn)],
                o_hbm.at[pl.ds(r0, nr), pl.ds(n0, nn)], os_.at[i])

        def wq(q, n0, nn):
            r0, c0 = _QUAD[q]
            return xw_vmem[pl.ds(r0 // 2, _H // 2), pl.ds(c0 + n0, nn)]

        def prod(i, p0, r, c, nt):
            a = pltpu.bitcast(sa_vmem[i - 1, pl.ds(p0 // 4, r // 2), :], _bf16)
            if i == 2:
                bb = wq(0, c * nt, nt)
            elif i == 5:
                bb = wq(3, c * nt, nt)
            else:
                bb = sb_vmem[_SBSLOT[i], :, pl.ds(c * nt, nt)]
            return jnp.dot(a, pltpu.bitcast(bb, _bf16), preferred_element_type=_f32)

        def put(val, p0, r, isq, cols):
            for i in range(r // _G):
                o_vmem[pl.ds(p0 + (2 * i + isq) * _G, _G), cols] = (
                    val[i * _G:(i + 1) * _G].astype(_bf16))

        gcp = pltpu.make_async_copy(g_hbm, g_vmem, gs.at[0])
        bcp = pltpu.make_async_copy(b_hbm, b_vmem, gs.at[1])
        g32 = b32 = None
        for op in ops:
            k = op[0]
            if k == "xstart":
                xcp(op[1]).start()
            elif k == "xwait":
                xcp(op[1]).wait()
            elif k == "wstart":
                wcp(op[1]).start()
            elif k == "wwait":
                wcp(op[1]).wait()
            elif k == "ostart":
                ocp(op[1]).start()
            elif k == "owait":
                ocp(op[1]).wait()
            elif k == "gstart":
                gcp.start()
                bcp.start()
            elif k == "fence":
                pl.semaphore_signal(fsem, 1)
                pl.semaphore_wait(fsem, 1)
            elif k == "gwait":
                gcp.wait()
                bcp.wait()
                g32 = g_vmem[...].astype(_f32).reshape(1, _D)
                b32 = b_vmem[...].astype(_f32).reshape(1, _D)
            elif k == "prep":
                _, i, n0, nn = op
                qa, qb, sign = _PREP[i]
                wa, wb = _unpack(wq(qa, n0, nn)), _unpack(wq(qb, n0, nn))
                sb_vmem[_SBSLOT[i], :, pl.ds(n0, nn)] = _pack(
                    *[wa[h] + wb[h] if sign > 0 else wa[h] - wb[h] for h in range(2)])
            elif k == "ln":
                _, r0, nr = op
                for gi in range(nr // _G):
                    rr = r0 + 2 * gi * _G
                    xp = _unpack(xw_vmem[pl.ds((xo + rr) // 2, _G // 2), :])
                    xq = _unpack(xw_vmem[pl.ds((xo + rr + _G) // 2, _G // 2), :])
                    lhs = []
                    for h in range(2):
                        yp, yq = _ln_f32(xp[h], g32, b32), _ln_f32(xq[h], g32, b32)
                        a11, a12, a21, a22 = yp[:, :_H], yp[:, _H:], yq[:, :_H], yq[:, _H:]
                        lhs.append((a11 + a22, a21 + a22, a11, a22,
                                    a11 + a12, a21 - a11, a12 - a22))
                    for i in range(7):
                        sa_vmem[i, pl.ds(rr // 4, _G // 2), :] = _pack(lhs[0][i], lhs[1][i])
            elif k == "mm":
                _, i, p0, r, c, nt, tb = op
                m = prod(i, p0, r, c, nt)
                left, right = pl.ds(c * nt, nt), pl.ds(_H + c * nt, nt)
                t11, t12, t21, t22 = (
                    t_vmem.at[tb * 4 + t, pl.ds(0, r), left] for t in range(4))
                if i == 2:
                    t21[...] = m
                    t22[...] = -m
                elif i == 5:
                    t12[...] = m
                    t11[...] = -m
                elif i == 1:
                    t11[...] = t11[...] + m
                    t22[...] = t22[...] + m
                elif i == 3:
                    put(t12[...] + m, p0, r, 0, right)
                    t22[...] = t22[...] + m
                elif i == 6:
                    put(t22[...] + m, p0, r, 1, right)
                elif i == 4:
                    put(t21[...] + m, p0, r, 1, left)
                    t11[...] = t11[...] + m
                elif i == 7:
                    put(t11[...] + m, p0, r, 0, left)
            else:
                raise ValueError(op)

    return kernel


@jax.jit
def pallas_standalone__layernorm_linear__prompt_kernel(x, g, b, w):
    bsz, seq, d = x.shape
    assert (bsz * seq, d, w.shape[1]) == (_M, _D, _N)
    ops, xch, wch, och = _schedule()
    anyspec = pl.BlockSpec(memory_space=pl.ANY)
    out = pl.pallas_call(
        _make_kernel(ops, xch, wch, och),
        grid=(),
        in_specs=[anyspec] * 4,
        out_specs=anyspec,
        out_shape=jax.ShapeDtypeStruct((_M, _N), x.dtype),
        scratch_shapes=[
            pltpu.VMEM(((_D + _M) // 2, _D), _u32),
            pltpu.VMEM((7, _M // 4, _H), _u32),
            pltpu.VMEM((5, _H // 2, _H), _u32),
            pltpu.VMEM((8, max(_REGIONS), _H), _f32),
            pltpu.VMEM((_M, _N), _bf16),
            pltpu.VMEM((_D,), _bf16),
            pltpu.VMEM((_D,), _bf16),
            pltpu.SemaphoreType.DMA((len(xch),)),
            pltpu.SemaphoreType.DMA((len(wch),)),
            pltpu.SemaphoreType.DMA((len(och),)),
            pltpu.SemaphoreType.DMA((2,)),
            pltpu.SemaphoreType.REGULAR,
        ],
        compiler_params=pltpu.CompilerParams(
            vmem_limit_bytes=64 * 1024 * 1024,
            flags={"XLA_TPU_EVENLY_DISTRIBUTE_CRITICAL_NODES": True},
        ),
        name="layernorm_linear",
    )(x.reshape(_M, _D), g, b, w)
    return out.reshape(bsz, seq, _N)
```
